```python
import os as _os
_os.environ.setdefault("JAX_PLATFORMS", "cpu")
import jax
import jax.numpy as jnp

def _softmax(x, axis=-1):
    return jax.nn.softmax(x, axis=axis)
def _gelu(x):
    return jax.nn.gelu(x, approximate=True)
def _silu(x):
    return jax.nn.silu(x)
def _sigmoid(x):
    return jax.nn.sigmoid(x)
def _layernorm(x, axis=-1, eps=1e-5):
    m = jnp.mean(x, axis=axis, keepdims=True)
    v = jnp.var(x, axis=axis, keepdims=True)
    return (x - m) / jnp.sqrt(v + eps)
def _scatter_add(tgt, idx, src, axis=0):
    return tgt.at[idx].add(src)
def _segment_sum(src, seg, n):
    return jax.ops.segment_sum(src, seg, n)
class _Rng:
    def __init__(self, key):
        self._k = key
    def _next(self):
        self._k, sub = jax.random.split(self._k)
        return sub
    def normal(self, shape):
        return jax.random.normal(self._next(), shape, dtype=jnp.bfloat16)
    def randint(self, lo, hi, shape):
        return jax.random.randint(self._next(), shape, lo, hi, dtype=jnp.int32)
    def uniform(self, shape, lo=0.0, hi=1.0):
        return jax.random.uniform(self._next(), shape, jnp.bfloat16, lo, hi)
    def permutation(self, n):
        return jax.random.permutation(self._next(), n)


kernel_name = 'parallel_sum__grouped_kv_mqa__dense_activation_silu__prompt'

def setup_inputs():
    _rng = _Rng(jax.random.key(int.from_bytes(__import__("os").urandom(4), "little")))
    _w = (lambda a: (lambda t: t.astype(jnp.bfloat16) if jnp.issubdtype(t.dtype, jnp.floating) else t)(jnp.asarray(a)))
    def _A_setup():
        B, S, D, H = 1, 2048, 512, 32
        Dh = D // H
        return {
            "x": _w((lambda *s: _rng.normal(s) * 0.05)(B, S, D)),
            "wq": _w((lambda *s: _rng.normal(s) * 0.05)(D, H * Dh)),
            "wk": _w((lambda *s: _rng.normal(s) * 0.05)(D, Dh)),
            "wv": _w((lambda *s: _rng.normal(s) * 0.05)(D, Dh)),
            "wo": _w((lambda *s: _rng.normal(s) * 0.05)(H * Dh, D)),
        }
    _A_in = _A_setup()

    def _B_setup():
        B, S, D, F = 1, 2048, 512, 1376
        return {
            "x": _w((lambda *s: _rng.normal(s) * 0.05)(B, S, D)),
            "w1": _w((lambda *s: _rng.normal(s) * 0.05)(D, F) * (D ** -0.5)),
            "w2": _w((lambda *s: _rng.normal(s) * 0.05)(F, D) * (F ** -0.5)),
        }
    _B_in = _B_setup()

    return {
        "A_x": _A_in["x"],
        "A_wq": _A_in["wq"],
        "A_wk": _A_in["wk"],
        "A_wv": _A_in["wv"],
        "A_wo": _A_in["wo"],
        "B_x": _B_in["x"],
        "B_w1": _B_in["w1"],
        "B_w2": _B_in["w2"],
    }

def reference(A_x, A_wq, A_wk, A_wv, A_wo, B_x, B_w1, B_w2):
    def _A_ref(x, wq, wk, wv, wo):
        B, S, D = x.shape
        H = 32
        Dh = D // H
        q = (lambda x, *d: x.transpose(*d))((x @ wq).reshape(B, S, H, Dh), 0, 2, 1, 3)
        k = x @ wk
        v = x @ wv
        scores = jnp.einsum("bhqd,bkd->bhqk", q, k) * (Dh ** -0.5)
        p = _softmax(scores, axis=-1)
        o = jnp.einsum("bhqk,bkd->bhqd", p, v)
        return (lambda x, *d: x.transpose(*d))(o, 0, 2, 1, 3).reshape(B, S, H * Dh) @ wo

    def _B_ref(x, w1, w2):
        h = jnp.einsum("bsd,df->bsf", x, w1)
        h = _silu(h)
        out = jnp.einsum("bsf,fd->bsd", h, w2)
        return out

    x = A_x
    xn = _layernorm(x, axis=-1)
    return x + _A_ref(xn, A_wq, A_wk, A_wv, A_wo) + _B_ref(xn, B_w1, B_w2)
```

```python
import functools

import jax
import jax.numpy as jnp
import jax.experimental.pallas as pl
import jax.experimental.pallas.tpu as pltpu

H = 32
TQ = 1024
CK = 512
HP = 2
LOG2E = 1.4426950408889634
SAFE_BOUND = 60.0


def _mm(a, b):
    return jnp.dot(a, b, preferred_element_type=jnp.float32)


def _mm_nt(a, b):
    return jax.lax.dot_general(a, b, (((1,), (1,)), ((), ())), preferred_element_type=jnp.float32)


def _kernel(x_ref, wq_ref, wk_ref, wv_ref, wo_hbm, w1_hbm, w2_hbm, o_ref,
            xn_ref, k_ref, vt_ref, kn_ref, qt_ref, ot_ref, res_ref,
            wo_ref, w1_ref, w2_ref, sems):
    S, D = x_ref.shape
    dh = D // H
    i = pl.program_id(0)
    cp1 = pltpu.make_async_copy(w1_hbm, w1_ref, sems.at[0])
    cp2 = pltpu.make_async_copy(w2_hbm, w2_ref, sems.at[1])
    cp3 = pltpu.make_async_copy(wo_hbm, wo_ref, sems.at[2])

    @pl.when(i == 0)
    def _():
        cp1.start()
        cp2.start()
        cp3.start()
        rb = 256
        for r in range(S // rb):
            x = x_ref[r * rb:(r + 1) * rb, :].astype(jnp.float32)
            m = jnp.mean(x, axis=-1, keepdims=True)
            xc = x - m
            v = jnp.mean(xc * xc, axis=-1, keepdims=True)
            xn_ref[r * rb:(r + 1) * rb, :] = (xc * jax.lax.rsqrt(v + 1e-5)).astype(jnp.bfloat16)
        xn = xn_ref[...]
        k = _mm_nt(xn, wk_ref[...]).astype(jnp.bfloat16)
        k_ref[...] = k
        kf = k.astype(jnp.float32)
        kn_ref[0] = jnp.max(jnp.sum(kf * kf, axis=-1, keepdims=True))
        vt_ref[...] = _mm_nt(wv_ref[...], xn).astype(jnp.bfloat16)

    row0 = pl.multiple_of(i * TQ, TQ)
    xt = xn_ref[pl.ds(row0, TQ), :]
    q = _mm(xt, wq_ref[...]) * (dh ** -0.5 * LOG2E)
    qt = q.T.astype(jnp.bfloat16)
    qt_ref[...] = qt
    qf = qt.astype(jnp.float32)
    qn = jnp.max(jnp.sum((qf * qf).reshape(H, dh, TQ), axis=1))
    safe = qn * kn_ref[0] < SAFE_BOUND * SAFE_BOUND

    @pl.when(i == 0)
    def _():
        cp1.wait()
        cp2.wait()

    hcur = _mm_nt(xt, w1_ref[...])
    hcur = hcur * jax.nn.sigmoid(hcur)
    ff = _mm(hcur.astype(jnp.bfloat16), w2_ref[...])
    res_ref[...] = x_ref[pl.ds(row0, TQ), :].astype(jnp.float32) + ff

    def head(h, use_max):
        hs = pl.ds(pl.multiple_of(h * dh, dh), dh)
        qh = qt_ref[hs, :]
        m = acc = l = None
        for j in range(S // CK):
            s = _mm(k_ref[j * CK:(j + 1) * CK, :], qh)
            if use_max:
                mj = jnp.max(s, axis=0, keepdims=True)
                mn = mj if m is None else jnp.maximum(m, mj)
                s = s - mn
            p = jnp.exp2(s)
            lj = jnp.sum(p.reshape(CK // 8, 8, TQ), axis=0)
            o = _mm(vt_ref[:, j * CK:(j + 1) * CK], p.astype(jnp.bfloat16))
            if acc is None:
                acc, l = o, lj
            elif use_max:
                a = jnp.exp2(m - mn)
                acc, l = acc * a + o, l * a + lj
            else:
                acc, l = acc + o, l + lj
            if use_max:
                m = mn
        ot_ref[hs, :] = acc / jnp.sum(l, axis=0, keepdims=True)

    def heads(g, c, use_max):
        for u in range(HP):
            head(g * HP + u, use_max)
        return c

    @pl.when(safe)
    def _():
        jax.lax.fori_loop(0, H // HP, functools.partial(heads, use_max=False), 0)

    @pl.when(jnp.logical_not(safe))
    def _():
        jax.lax.fori_loop(0, H // HP, functools.partial(heads, use_max=True), 0)

    @pl.when(i == 0)
    def _():
        cp3.wait()

    att = _mm(ot_ref[...].T.astype(jnp.bfloat16), wo_ref[...])
    o_ref[...] = (res_ref[...] + att).astype(o_ref.dtype)


@jax.jit
def pallas_parallel_sum__grouped_kv_mqa__dense_activation_silu__prompt_kernel(
    A_x, A_wq, A_wk, A_wv, A_wo, B_x, B_w1, B_w2,
):
    del B_x
    B, S, D = A_x.shape
    dh = D // H
    x = A_x.reshape(B * S, D)
    A_wk, A_wv, B_w1 = A_wk.T, A_wv.T, B_w1.T
    full = lambda a: pl.BlockSpec(a.shape, lambda i: (0, 0))
    out = pl.pallas_call(
        _kernel,
        grid=(S // TQ,),
        in_specs=[full(a) for a in (x, A_wq, A_wk, A_wv)]
        + [pl.BlockSpec(memory_space=pl.ANY)] * 3,
        out_specs=pl.BlockSpec((TQ, D), lambda i: (i, 0)),
        out_shape=jax.ShapeDtypeStruct((S, D), A_x.dtype),
        scratch_shapes=[
            pltpu.VMEM((S, D), jnp.bfloat16),
            pltpu.VMEM((S, dh), jnp.bfloat16),
            pltpu.VMEM((dh, S), jnp.bfloat16),
            pltpu.SMEM((1,), jnp.float32),
            pltpu.VMEM((D, TQ), jnp.bfloat16),
            pltpu.VMEM((D, TQ), jnp.float32),
            pltpu.VMEM((TQ, D), jnp.float32),
            pltpu.VMEM(A_wo.shape, A_wo.dtype),
            pltpu.VMEM(B_w1.shape, B_w1.dtype),
            pltpu.VMEM(B_w2.shape, B_w2.dtype),
            pltpu.SemaphoreType.DMA((3,)),
        ],
        compiler_params=pltpu.CompilerParams(
            dimension_semantics=("arbitrary",), vmem_limit_bytes=100 * 2**20),
    )(x, A_wq, A_wk, A_wv, A_wo, B_w1, B_w2)
    return out.reshape(B, S, D)
```
